```python
import jax
import jax.numpy as jnp

def _softmax(x, axis=-1):
    return jax.nn.softmax(x, axis=axis)

def _gelu(x):
    return jax.nn.gelu(x, approximate=True)

def _silu(x):
    return jax.nn.silu(x)

def _sigmoid(x):
    return jax.nn.sigmoid(x)

def _layernorm(x, axis=-1, eps=1e-05):
    m = jnp.mean(x, axis=axis, keepdims=True)
    v = jnp.var(x, axis=axis, keepdims=True)
    return (x - m) / jnp.sqrt(v + eps)

def _scatter_add(tgt, idx, src, axis=0):
    return tgt.at[idx].add(src)

def _segment_sum(src, seg, n):
    return jax.ops.segment_sum(src, seg, n)

class _Rng:

    def __init__(self, key):
        self._k = key

    def _next(self):
        self._k, sub = jax.random.split(self._k)
        return sub

    def normal(self, shape):
        return jax.random.normal(self._next(), shape, dtype=jnp.bfloat16)

    def randint(self, lo, hi, shape):
        return jax.random.randint(self._next(), shape, lo, hi, dtype=jnp.int32)

    def uniform(self, shape, lo=0.0, hi=1.0):
        return jax.random.uniform(self._next(), shape, jnp.bfloat16, lo, hi)

    def permutation(self, n):
        return jax.random.permutation(self._next(), n)
kernel_name = 'standalone__dilated_atrous__vision'

def setup_inputs():
    _rng = _Rng(jax.random.key(int.from_bytes(__import__("os").urandom(4), "little")))
    _w = lambda a: (lambda t: t.astype(jnp.bfloat16) if jnp.issubdtype(t.dtype, jnp.floating) else t)(jnp.asarray(a))
    H = W = 384
    C = 384
    k = 1
    return {'x': _w((lambda *s: _rng.normal(s) * 0.05)(1, H, W, C)), 'w': _w((lambda *s: _rng.normal(s) * 0.05)(k, k, C, C) * (1.0 / (k * C ** 0.5)))}

def reference(x, w):
    B, H, W, C = x.shape
    k = 1
    rate = 2
    pad = (k - 1) * rate // 2
    xp = jnp.pad(x, ((0, 0), (pad, pad), (pad, pad), (0, 0)))
    out = jnp.zeros_like(x)
    for i in range(k):
        for j in range(k):
            tap = xp[:, i * rate:i * rate + H, j * rate:j * rate + W, :].copy()
            out = out + jnp.einsum('bhwc,co->bhwo', tap, w[i, j])
    return out
```

```python
import jax
import jax.numpy as jnp
import jax.experimental.pallas as pl
import jax.experimental.pallas.tpu as pltpu


_K = 6
_RW = 48
_RS = 384
_SWITCH = 41
_WR_PER_STEP = 13
_LEAD = 16


@jax.jit
def pallas_standalone__dilated_atrous__vision_kernel(
    x: jax.Array,
    w: jax.Array,
):
    B, H, W, C = x.shape
    CO = w.shape[-1]
    assert C == CO and w.shape[0] == 1 and w.shape[1] == 1
    M = B * H * W
    K, RW, RS = _K, _RW, _RS
    MR = M // K
    nsteps = MR // RS
    nwr = MR // RW
    wps = RS // RW
    assert K * MR == M and nsteps * RS == MR and wps * RW == RS
    x3 = x.reshape(K, MR, C)
    w2 = w.reshape(C, CO)

    def kernel(x_hbm, w_ref, o_hbm, buf, wsem):
        def wr(j):
            off = pl.multiple_of(j * RW, RW)
            return pltpu.make_async_copy(
                buf.at[:, pl.ds(off, RW), :], o_hbm.at[:, pl.ds(off, RW), :], wsem)

        def start_wr(j, c):
            wr(j).start()
            return c

        def compute(i):
            off = pl.multiple_of(i * RS, RS)
            xv = buf[:, pl.ds(off, RS), :].reshape(K * RS, C)
            y = jnp.dot(xv, w_ref[...], preferred_element_type=jnp.float32)
            buf[:, pl.ds(off, RS), :] = y.astype(buf.dtype).reshape(K, RS, CO)

        def main(rsem):
            def rd(i):
                off = pl.multiple_of(i * RS, RS)
                return pltpu.make_async_copy(
                    x_hbm.at[:, pl.ds(off, RS), :], buf.at[:, pl.ds(off, RS), :],
                    rsem.at[i])

            def start_rd(i, c):
                rd(i).start()
                return c

            def wait_rd(i, c):
                rd(i).wait()
                return c

            jax.lax.fori_loop(0, nsteps, start_rd, 0)

            def step1(i, c):
                rd(i).wait()
                compute(i)
                return c

            jax.lax.fori_loop(0, _SWITCH, step1, 0)
            jax.lax.fori_loop(_SWITCH, nsteps - 1, wait_rd, 0)
            jax.lax.fori_loop(0, _LEAD, start_wr, 0)
            jax.lax.fori_loop(nsteps - 1, nsteps, wait_rd, 0)

            def step2(i, nxt):
                hi = jnp.minimum(nxt + _WR_PER_STEP, i * wps)
                jax.lax.fori_loop(nxt, hi, start_wr, 0)
                compute(i)
                return hi

            nxt = jax.lax.fori_loop(_SWITCH, nsteps, step2, _LEAD)
            jax.lax.fori_loop(nxt, nwr, start_wr, 0)

        pl.run_scoped(main, pltpu.SemaphoreType.DMA((nsteps,)))
        pltpu.make_async_copy(buf, o_hbm, wsem).wait()

    out = pl.pallas_call(
        kernel,
        in_specs=[pl.BlockSpec(memory_space=pl.ANY),
                  pl.BlockSpec(memory_space=pltpu.VMEM)],
        out_specs=pl.BlockSpec(memory_space=pl.ANY),
        out_shape=jax.ShapeDtypeStruct((K, MR, CO), x.dtype),
        scratch_shapes=[pltpu.VMEM((K, MR, C), x.dtype),
                        pltpu.SemaphoreType.DMA(())],
        compiler_params=pltpu.CompilerParams(vmem_limit_bytes=120 * 1024 * 1024),
    )(x3, w2)
    return out.reshape(B, H, W, CO)
```

```python
import functools

import jax
import jax.numpy as jnp
import jax.experimental.pallas as pl
import jax.experimental.pallas.tpu as pltpu


_K = 6
_RW = 48
_RS = 192
_RR = 32
_PB = 12
_P0 = 36
_D = 13
_SWITCH = 57
_LEAD = 16
_WR_PER_STEP = 7


@jax.jit
def pallas_standalone__dilated_atrous__vision_kernel(
    x: jax.Array,
    w: jax.Array,
):
    B, H, W, C = x.shape
    CO = w.shape[-1]
    assert C == CO and w.shape[0] == 1 and w.shape[1] == 1
    M = B * H * W
    K, RW, RS, RR = _K, _RW, _RS, _RR
    KH = K // 2
    MR = M // K
    nsteps = MR // RS
    nwr = MR // RW
    npairs = MR // RR
    wps = RS // RW
    pps = RS // RR
    assert K * MR == M and nsteps * RS == MR and wps * RW == RS and pps * RR == RS
    assert _D >= pps and _P0 >= pps and _LEAD <= _SWITCH * wps
    x3 = x.reshape(K, MR, C)
    w2 = w.reshape(C, CO)

    def kernel(x_hbm, w_hbm, o_hbm, buf, w_ref, wsem, wtsem):
        w_copy = pltpu.make_async_copy(w_hbm, w_ref, wtsem)
        w_copy.start()

        def start_wr(j, c):
            off = pl.multiple_of(j * RW, RW)
            pltpu.make_async_copy(
                buf.at[:, pl.ds(off, RW), :], o_hbm.at[:, pl.ds(off, RW), :], wsem
            ).start()
            return c

        def compute(i):
            off = pl.multiple_of(i * RS, RS)
            xv = buf[:, pl.ds(off, RS), :].reshape(K * RS, C)
            y = jnp.dot(xv, w_ref[...], preferred_element_type=jnp.float32)
            buf[:, pl.ds(off, RS), :] = y.astype(buf.dtype).reshape(K, RS, CO)

        def main(rsem):
            def start_pair(p, c, second_priority=0):
                off = pl.multiple_of(p * RR, RR)
                sem = rsem.at[p // pps]
                pltpu.make_async_copy(
                    x_hbm.at[0:KH, pl.ds(off, RR), :],
                    buf.at[0:KH, pl.ds(off, RR), :], sem).start(priority=1)
                pltpu.make_async_copy(
                    x_hbm.at[KH:K, pl.ds(off, RR), :],
                    buf.at[KH:K, pl.ds(off, RR), :], sem
                ).start(priority=second_priority)
                return c

            def wait_step(i, c):
                off = pl.multiple_of(i * RS, RS)
                pltpu.make_async_copy(
                    x_hbm.at[:, pl.ds(off, RS), :], buf.at[:, pl.ds(off, RS), :],
                    rsem.at[i]).wait()
                return c

            jax.lax.fori_loop(
                0, _PB, functools.partial(start_pair, second_priority=1), 0)
            jax.lax.fori_loop(_PB, _P0, start_pair, 0)
            w_copy.wait()

            def step1(i, nxt):
                hi = jnp.minimum(nxt + _D, npairs)
                jax.lax.fori_loop(nxt, hi, start_pair, 0)
                wait_step(i, 0)
                compute(i)
                return hi

            nxt = jax.lax.fori_loop(0, _SWITCH, step1, _P0)
            jax.lax.fori_loop(nxt, npairs, start_pair, 0)

            jax.lax.fori_loop(_SWITCH, nsteps - 1, wait_step, 0)
            jax.lax.fori_loop(0, _LEAD, start_wr, 0)
            jax.lax.fori_loop(nsteps - 1, nsteps, wait_step, 0)

            def step2(i, nxt):
                hi = jnp.minimum(nxt + _WR_PER_STEP, i * wps)
                jax.lax.fori_loop(nxt, hi, start_wr, 0)
                compute(i)
                return hi

            nxt = jax.lax.fori_loop(_SWITCH, nsteps, step2, _LEAD)
            jax.lax.fori_loop(nxt, nwr, start_wr, 0)

        pl.run_scoped(main, pltpu.SemaphoreType.DMA((nsteps,)))
        pltpu.make_async_copy(buf, o_hbm, wsem).wait()

    out = pl.pallas_call(
        kernel,
        in_specs=[pl.BlockSpec(memory_space=pl.ANY),
                  pl.BlockSpec(memory_space=pl.ANY)],
        out_specs=pl.BlockSpec(memory_space=pl.ANY),
        out_shape=jax.ShapeDtypeStruct((K, MR, CO), x.dtype),
        scratch_shapes=[pltpu.VMEM((K, MR, C), x.dtype),
                        pltpu.VMEM((C, CO), w.dtype),
                        pltpu.SemaphoreType.DMA(()),
                        pltpu.SemaphoreType.DMA(())],
        compiler_params=pltpu.CompilerParams(vmem_limit_bytes=120 * 1024 * 1024),
    )(x3, w2)
    return out.reshape(B, H, W, CO)
```

```python
import jax
import jax.numpy as jnp
import jax.experimental.pallas as pl
import jax.experimental.pallas.tpu as pltpu


_K = 6
_S = 2048
_RS = 128
_RR = 8
_WSIZES = (40, 40, 48)
_LOOKAHEAD = 3
_SWITCH = 93
_LEAD = 6
_WG_PER_STEP = 2


@jax.jit
def pallas_standalone__dilated_atrous__vision_kernel(
    x: jax.Array,
    w: jax.Array,
):
    B, H, W, C = x.shape
    CO = w.shape[-1]
    assert C == CO and w.shape[0] == 1 and w.shape[1] == 1
    M = B * H * W
    K, S, RS, RR = _K, _S, _RS, _RR
    NB = M // (K * S)
    HB = NB // 2
    spb = S // RS
    shift = spb.bit_length() - 1
    nsteps = NB * spb
    hs = nsteps // 2
    assert NB * K * S == M and NB % 2 == 0 and HB >= 2
    assert spb == 1 << shift and RS % RR == 0 and sum(_WSIZES) == RS
    assert _SWITCH + _LOOKAHEAD <= hs and _LEAD <= _SWITCH
    x4 = x.reshape(NB, K, S, C)
    w2 = w.reshape(C, CO)

    def kernel(x_hbm, w_hbm, o_hbm, buf, w_ref, out_sem, w_sem):
        w_copy = pltpu.make_async_copy(w_hbm, w_ref, w_sem)
        w_copy.start()

        def loc(i):
            if isinstance(i, int):
                return i >> shift, (i & (spb - 1)) * RS
            b = jax.lax.shift_right_logical(i, shift)
            return b, pl.multiple_of((i & (spb - 1)) * RS, RS)

        def start_write_group(i, c):
            b, off = loc(i)
            o = 0
            for r in _WSIZES:
                pltpu.make_async_copy(
                    buf.at[b, :, pl.ds(off + o, r), :],
                    o_hbm.at[b, :, pl.ds(off + o, r), :], out_sem).start()
                o += r
            return c

        def compute(i):
            b, off = loc(i)
            xv = buf[b, :, pl.ds(off, RS), :].reshape(K * RS, C)
            y = jnp.dot(xv, w_ref[...], preferred_element_type=jnp.float32)
            buf[b, :, pl.ds(off, RS), :] = y.astype(buf.dtype).reshape(K, RS, CO)

        def main(first_sems, second_sems):
            def read(b, off, n, sem):
                return pltpu.make_async_copy(
                    x_hbm.at[b, :, pl.ds(off, n), :],
                    buf.at[b, :, pl.ds(off, n), :], sem)

            def start_read_group(g, c=0, first_priority=0):
                b, off = loc(g)
                if isinstance(g, int):
                    k = int(g >= hs - spb) + int(g == hs - 1)
                else:
                    k = ((g >= hs - spb).astype(jnp.int32)
                         + (g == hs - 1).astype(jnp.int32))
                for q in range(RS // RR):
                    o = off + q * RR
                    if not isinstance(o, int):
                        o = pl.multiple_of(o, RR)
                    read(b + HB, o, RR, second_sems.at[k]).start(priority=1)
                    read(b, o, RR, first_sems.at[g]).start(priority=first_priority)
                return c

            def wait_first(i, c):
                b, off = loc(i)
                read(b, off, RS, first_sems.at[i]).wait()
                return c

            for g in range(_LOOKAHEAD):
                start_read_group(g, first_priority=1 if g == 0 else 0)
            w_copy.wait()

            def step1(i, c):
                start_read_group(i + _LOOKAHEAD)
                wait_first(i, 0)
                compute(i)
                return c

            jax.lax.fori_loop(0, _SWITCH, step1, 0)
            for g in range(_SWITCH + _LOOKAHEAD, hs):
                start_read_group(g)
            jax.lax.fori_loop(_SWITCH, hs, wait_first, 0)
            pltpu.make_async_copy(
                x_hbm.at[pl.ds(HB, HB - 1)], buf.at[pl.ds(HB, HB - 1)],
                second_sems.at[0]).wait()
            read(NB - 1, 0, S - RS, second_sems.at[1]).wait()
            jax.lax.fori_loop(0, _LEAD, start_write_group, 0)
            read(NB - 1, S - RS, RS, second_sems.at[2]).wait()

            def step2(i, nxt):
                hi = jnp.minimum(nxt + _WG_PER_STEP, i)
                jax.lax.fori_loop(nxt, hi, start_write_group, 0)
                compute(i)
                return hi

            nxt = jax.lax.fori_loop(_SWITCH, nsteps, step2, _LEAD)
            jax.lax.fori_loop(nxt, nsteps, start_write_group, 0)

        pl.run_scoped(main, pltpu.SemaphoreType.DMA((hs,)),
                      pltpu.SemaphoreType.DMA((3,)))
        pltpu.make_async_copy(buf, o_hbm, out_sem).wait()

    out = pl.pallas_call(
        kernel,
        in_specs=[pl.BlockSpec(memory_space=pl.ANY),
                  pl.BlockSpec(memory_space=pl.ANY)],
        out_specs=pl.BlockSpec(memory_space=pl.ANY),
        out_shape=jax.ShapeDtypeStruct((NB, K, S, CO), x.dtype),
        scratch_shapes=[pltpu.VMEM((NB, K, S, C), x.dtype),
                        pltpu.VMEM((C, CO), w.dtype),
                        pltpu.SemaphoreType.DMA(()),
                        pltpu.SemaphoreType.DMA(())],
        compiler_params=pltpu.CompilerParams(
            vmem_limit_bytes=120 * 1024 * 1024,
            disable_bounds_checks=True),
    )(x4, w2)
    return out.reshape(B, H, W, CO)
```

```python
import jax
import jax.numpy as jnp
import jax.experimental.pallas as pl
import jax.experimental.pallas.tpu as pltpu


_K = 6
_S = 2048
_RS = 128
_RR = 16
_RK = 3
_WSIZES = (32, 48, 48)
_LOOKAHEAD = 3
_SWITCH = 93
_TAIL = 96
_LEAD = 6
_WG_PER_STEP = 2


@jax.jit
def pallas_standalone__dilated_atrous__vision_kernel(
    x: jax.Array,
    w: jax.Array,
):
    B, H, W, C = x.shape
    CO = w.shape[-1]
    assert C == CO and w.shape[0] == 1 and w.shape[1] == 1
    M = B * H * W
    K, S, RS, RR, RK = _K, _S, _RS, _RR, _RK
    NB = M // (K * S)
    HB = NB // 2
    spb = S // RS
    shift = spb.bit_length() - 1
    nsteps = NB * spb
    hs = nsteps // 2
    assert NB * K * S == M and NB % 2 == 0 and HB >= 2
    assert spb == 1 << shift and RS % RR == 0 and K % RK == 0
    assert sum(_WSIZES) == RS and 0 < _TAIL <= RS and _TAIL % RR == 0
    assert _SWITCH + _LOOKAHEAD <= hs and _LEAD <= _SWITCH
    x4 = x.reshape(NB, K, S, C)
    w2 = w.reshape(C, CO)

    def kernel(x_hbm, w_hbm, o_hbm, buf, w_ref, out_sem, w_sem):
        w_copy = pltpu.make_async_copy(w_hbm, w_ref, w_sem)
        w_copy.start()

        def loc(i):
            if isinstance(i, int):
                return i >> shift, (i & (spb - 1)) * RS
            b = jax.lax.shift_right_logical(i, shift)
            return b, pl.multiple_of((i & (spb - 1)) * RS, RS)

        def start_write_group(i, c):
            b, off = loc(i)
            o = 0
            for r in _WSIZES:
                pltpu.make_async_copy(
                    buf.at[b, :, pl.ds(off + o, r), :],
                    o_hbm.at[b, :, pl.ds(off + o, r), :], out_sem).start()
                o += r
            return c

        def compute(i):
            b, off = loc(i)
            xv = buf[b, :, pl.ds(off, RS), :].reshape(K * RS, C)
            y = jnp.dot(xv, w_ref[...], preferred_element_type=jnp.float32)
            buf[b, :, pl.ds(off, RS), :] = y.astype(buf.dtype).reshape(K, RS, CO)

        def main(first_sems, second_sems):
            def read(b, k0, nk, off, n, sem):
                return pltpu.make_async_copy(
                    x_hbm.at[b, k0:k0 + nk, pl.ds(off, n), :],
                    buf.at[b, k0:k0 + nk, pl.ds(off, n), :], sem)

            def start_read_group(g, first_priority=0):
                b, off = loc(g)
                if isinstance(g, int):
                    head = int(g >= hs - spb)
                    tail = head + int(g == hs - 1)
                else:
                    head = (g >= hs - spb).astype(jnp.int32)
                    tail = head + (g == hs - 1).astype(jnp.int32)
                for r0 in range(0, RS, RR):
                    o = off + r0
                    if not isinstance(o, int):
                        o = pl.multiple_of(o, RR)
                    second = second_sems.at[tail if r0 >= RS - _TAIL else head]
                    for k0 in range(0, K, RK):
                        read(b + HB, k0, RK, o, RR, second).start(priority=1)
                        read(b, k0, RK, o, RR, first_sems.at[g]).start(
                            priority=first_priority)

            def wait_first(i, c):
                b, off = loc(i)
                read(b, 0, K, off, RS, first_sems.at[i]).wait()
                return c

            for g in range(_LOOKAHEAD):
                start_read_group(g, first_priority=1 if g == 0 else 0)
            w_copy.wait()

            def step1(i, c):
                start_read_group(i + _LOOKAHEAD)
                wait_first(i, 0)
                compute(i)
                return c

            jax.lax.fori_loop(0, _SWITCH, step1, 0)
            for g in range(_SWITCH + _LOOKAHEAD, hs):
                start_read_group(g)
            jax.lax.fori_loop(_SWITCH, hs, wait_first, 0)
            pltpu.make_async_copy(
                x_hbm.at[pl.ds(HB, HB - 1)], buf.at[pl.ds(HB, HB - 1)],
                second_sems.at[0]).wait()
            read(NB - 1, 0, K, 0, S - _TAIL, second_sems.at[1]).wait()
            jax.lax.fori_loop(0, _LEAD, start_write_group, 0)
            read(NB - 1, 0, K, S - _TAIL, _TAIL, second_sems.at[2]).wait()

            def step2(i, nxt):
                hi = jnp.minimum(nxt + _WG_PER_STEP, i)
                jax.lax.fori_loop(nxt, hi, start_write_group, 0)
                compute(i)
                return hi

            nxt = jax.lax.fori_loop(_SWITCH, nsteps, step2, _LEAD)
            jax.lax.fori_loop(nxt, nsteps, start_write_group, 0)

        pl.run_scoped(main, pltpu.SemaphoreType.DMA((hs,)),
                      pltpu.SemaphoreType.DMA((3,)))
        pltpu.make_async_copy(buf, o_hbm, out_sem).wait()

    out = pl.pallas_call(
        kernel,
        in_specs=[pl.BlockSpec(memory_space=pl.ANY),
                  pl.BlockSpec(memory_space=pl.ANY)],
        out_specs=pl.BlockSpec(memory_space=pl.ANY),
        out_shape=jax.ShapeDtypeStruct((NB, K, S, CO), x.dtype),
        scratch_shapes=[pltpu.VMEM((NB, K, S, C), x.dtype),
                        pltpu.VMEM((C, CO), w.dtype),
                        pltpu.SemaphoreType.DMA(()),
                        pltpu.SemaphoreType.DMA(())],
        compiler_params=pltpu.CompilerParams(
            vmem_limit_bytes=120 * 1024 * 1024,
            disable_bounds_checks=True),
    )(x4, w2)
    return out.reshape(B, H, W, CO)
```
